```python
import os as _os
_os.environ.setdefault("JAX_PLATFORMS", "cpu")
import jax
import jax.numpy as jnp

def _softmax(x, axis=-1):
    return jax.nn.softmax(x, axis=axis)
def _gelu(x):
    return jax.nn.gelu(x, approximate=True)
def _silu(x):
    return jax.nn.silu(x)
def _sigmoid(x):
    return jax.nn.sigmoid(x)
def _layernorm(x, axis=-1, eps=1e-5):
    m = jnp.mean(x, axis=axis, keepdims=True)
    v = jnp.var(x, axis=axis, keepdims=True)
    return (x - m) / jnp.sqrt(v + eps)
def _scatter_add(tgt, idx, src, axis=0):
    return tgt.at[idx].add(src)
def _segment_sum(src, seg, n):
    return jax.ops.segment_sum(src, seg, n)
class _Rng:
    def __init__(self, key):
        self._k = key
    def _next(self):
        self._k, sub = jax.random.split(self._k)
        return sub
    def normal(self, shape):
        return jax.random.normal(self._next(), shape, dtype=jnp.bfloat16)
    def randint(self, lo, hi, shape):
        return jax.random.randint(self._next(), shape, lo, hi, dtype=jnp.int32)
    def uniform(self, shape, lo=0.0, hi=1.0):
        return jax.random.uniform(self._next(), shape, jnp.bfloat16, lo, hi)
    def permutation(self, n):
        return jax.random.permutation(self._next(), n)


kernel_name = 'interleave_layers__linear_attn_block__mha_block__prompt'

def setup_inputs():
    _rng = _Rng(jax.random.key(int.from_bytes(__import__("os").urandom(4), "little")))
    _w = (lambda a: (lambda t: t.astype(jnp.bfloat16) if jnp.issubdtype(t.dtype, jnp.floating) else t)(jnp.asarray(a)))
    def _A_setup():
        B, S, D = 1, 2048, 640
        return {
            "x": _w((lambda *s: _rng.normal(s) * 0.05)(B, S, D)),
            "wqkv": _w((lambda *s: _rng.normal(s) * 0.1)(D, 3 * D)),
            "wo": _w((lambda *s: _rng.normal(s) * 0.05)(D, D)),
        }
    _A_in = _A_setup()

    def _B_setup():
        B, S, D, H = 1, 2048, 640, 32
        return {
            "x": _w((lambda *s: _rng.normal(s) * 0.05)(B, S, D)),
            "wqkv": _w((lambda *s: _rng.normal(s) * 0.1)(D, 3 * D)),
            "wo": _w((lambda *s: _rng.normal(s) * 0.05)(D, D)),
        }
    _B_in = _B_setup()

    return {
        "A_x": _A_in["x"],
        "A_wqkv": _A_in["wqkv"],
        "A_wo": _A_in["wo"],
        "B_x": _B_in["x"],
        "B_wqkv": _B_in["wqkv"],
        "B_wo": _B_in["wo"],
    }

def reference(A_x, A_wqkv, A_wo, B_x, B_wqkv, B_wo):
    def _A_ref(x, wqkv, wo):
        B, S, D = x.shape
        H = 32; Dh = D // H
        qkv = (lambda x, *d: x.transpose(*d))((x @ wqkv).reshape(B, S, 3, H, Dh), 2, 0, 3, 1, 4)
        q, k, v = qkv[0], qkv[1], qkv[2]
        phi = lambda t: jnp.where(t > 0, t + 1, jnp.exp(t)) + 1e-6
        pq, pk = phi(q), phi(k)
        kv = jnp.einsum("bhsd,bhse->bhde", pk, v)
        z = jnp.einsum("bhsd->bhd", pk)
        num = jnp.einsum("bhqd,bhde->bhqe", pq, kv)
        den = jnp.einsum("bhqd,bhd->bhq", pq, z)[..., None] + 1e-6
        o = num / den
        return (lambda x, *d: x.transpose(*d))(o, 0, 2, 1, 3).reshape(B, S, D) @ wo

    def _B_ref(x, wqkv, wo):
        B, S, D = x.shape
        H = 32
        Dh = D // H
        qkv = (lambda x, *d: x.transpose(*d))((x @ wqkv).reshape(B, S, 3, H, Dh), 2, 0, 3, 1, 4)
        q, k, v = qkv[0], qkv[1], qkv[2]
        scores = jnp.einsum("bhqd,bhkd->bhqk", q, k) * (Dh ** -0.5)
        p = _softmax(scores, axis=-1)
        o = jnp.einsum("bhqk,bhkd->bhqd", p, v)
        return (lambda x, *d: x.transpose(*d))(o, 0, 2, 1, 3).reshape(B, S, D) @ wo

    x = A_x
    x = x + _A_ref(_layernorm(x, axis=-1), A_wqkv, A_wo)
    x = x + _B_ref(_layernorm(x, axis=-1), B_wqkv, B_wo)
    x = x + _A_ref(_layernorm(x, axis=-1), A_wqkv, A_wo)
    x = x + _B_ref(_layernorm(x, axis=-1), B_wqkv, B_wo)
    return x
```

```python
import math

import jax
import jax.numpy as jnp
from jax import lax
import jax.experimental.pallas as pl
import jax.experimental.pallas.tpu as pltpu

S = 2048
D = 640
H = 32
DH = 20
LANE = 128
NG = D // LANE
TM = 512
TQ = 512
CH = 128
SK = 2
NQT = S // TQ
EB = 160

F32 = jnp.float32
BF16 = jnp.bfloat16
I32 = jnp.int32
I8 = jnp.int8

QA = 14.0
RADIX = QA * QA
XMAX = RADIX * 9 + 97
MAGIC = 1.5 * 2.0 ** 23

_NT = (((1,), (1,)), ((), ()))
_TN = (((0,), (0,)), ((), ()))

_STRADDLE = [h for h in range(H) if (DH * h) // LANE != (DH * h + DH - 1) // LANE]


def _layernorm(x):
    m = jnp.mean(x, axis=-1, keepdims=True)
    xc = x - m
    v = jnp.mean(xc * xc, axis=-1, keepdims=True)
    return xc * lax.rsqrt(v + 1e-5)


def _phi(t):
    return jnp.where(t > 0, t + 1.0, jnp.exp(t)) + 1e-6


def _pair_rows(even, odd):
    n = even.shape[1]
    row = lax.broadcasted_iota(jnp.int32, (8, n), 0)
    mid = jnp.where(row < 4, even[16:24], odd[0:8])
    return jnp.concatenate([even[0:16], mid, odd[8:24]], axis=0)


def _limbs(blk):
    n = blk.shape[1]
    row = lax.broadcasted_iota(I32, (8, n), 0)
    lo = row < 4
    a = jnp.abs(blk)
    me = jnp.maximum(jnp.maximum(a[0:8], a[8:16]), jnp.where(lo, a[16:24], 0.0))
    mo = jnp.maximum(jnp.maximum(a[24:32], a[32:40]), jnp.where(lo, 0.0, a[16:24]))
    me = jnp.max(me, axis=0, keepdims=True)
    mo = jnp.max(mo, axis=0, keepdims=True)
    se = XMAX / jnp.maximum(me, 1e-30)
    so = XMAX / jnp.maximum(mo, 1e-30)
    y = jnp.concatenate([blk[0:16] * se, blk[16:24] * jnp.where(lo, se, so), blk[24:40] * so], axis=0)
    tm = y * (1.0 / RADIX) + MAGIC
    r = y - (tm - MAGIC) * RADIX
    t = pltpu.bitcast(tm, I32)
    b = pltpu.bitcast(r + MAGIC, I32)
    m = pltpu.bitcast(r * (1.0 / QA) + MAGIC, I32)
    return (t * int(QA), t, b, m), me, mo


def _pack4(xs):
    return pltpu.bitcast(pltpu.pack_elementwise(xs, packed_dtype=I8), I32)


def _kernel(x_ref, wa_ref, woa_ref, wb_ref, wob_ref, o_ref,
            xres, wavt, wbt, k8, qw, ki, xs, cq_s, cks, ckc, vt, ot, sbuf, pq_s, pk_s, kvt_s):
    xres[...] = x_ref[...].astype(F32)
    for j in range(NG):
        cs = slice(j * LANE, (j + 1) * LANE)
        wavt[cs, :] = wa_ref[:, 2 * D + j * LANE:2 * D + (j + 1) * LANE].astype(F32).T.astype(BF16)
        wbt[cs, :] = wb_ref[:, cs].astype(F32).T.astype(BF16)
        wbt[D + j * LANE:D + (j + 1) * LANE, :] = (
            wb_ref[:, 2 * D + j * LANE:2 * D + (j + 1) * LANE].astype(F32).T.astype(BF16))
        wbt[2 * D + j * LANE:2 * D + (j + 1) * LANE, :] = (
            wb_ref[:, D + j * LANE:D + (j + 1) * LANE].astype(F32).T.astype(BF16))
    qw[D:D + 8, :] = jnp.zeros((8, S), I32)
    cks[...] = jnp.zeros(cks.shape, F32)
    vt[D:D + 8, :] = jnp.ones((8, S), F32)

    def out_proj(wo_ref):
        def body(t, c):
            rs = pl.ds(pl.multiple_of(t * TM, TM), TM)
            y = lax.dot_general(ot[:, rs], wo_ref[...], _TN, preferred_element_type=F32)
            xres[rs, :] = xres[rs, :] + y
            return c
        lax.fori_loop(0, S // TM, body, 0)

    def layer_a():
        def proj(t, c):
            rs = pl.ds(pl.multiple_of(t * TM, TM), TM)
            xn = _layernorm(xres[rs, :]).astype(BF16)
            qk = jnp.dot(xn, wa_ref[:, 0:2 * D], preferred_element_type=F32)
            pq_s[rs, :] = _phi(qk[:, 0:D]).astype(BF16)
            pk_s[rs, :] = _phi(qk[:, D:2 * D]).astype(BF16)
            vt[0:D, rs] = lax.dot_general(wavt[...], xn, _NT, preferred_element_type=F32)
            return c
        lax.fori_loop(0, S // TM, proj, 0)

        for i in range(4):
            lhs = jnp.concatenate([vt[EB * i:EB * (i + 1), :], vt[D:D + 8, :]], axis=0).astype(BF16)
            kv = jnp.dot(lhs, pk_s[:, LANE * i:LANE * i + 2 * LANE], preferred_element_type=F32)
            r = lax.broadcasted_iota(jnp.int32, kv.shape, 0)
            d = lax.broadcasted_iota(jnp.int32, kv.shape, 1) + (LANE * i - EB * i)
            hr = jnp.where(r < EB, r // DH, r - EB) * DH
            keep = jnp.logical_and(d >= hr, d < hr + DH)
            kvt_s[i] = jnp.where(keep, kv, 0.0).astype(BF16)

        def apply(t, c):
            rs = pl.ds(pl.multiple_of(t * TM, TM), TM)
            for i in range(4):
                n = lax.dot_general(kvt_s[i], pq_s[rs, LANE * i:LANE * i + 2 * LANE], _NT,
                                    preferred_element_type=F32)
                rden = 1.0 / (n[EB:EB + 8] + 1e-6)
                for p in range(4):
                    ev = n[40 * p:40 * p + 24] * rden[2 * p:2 * p + 1]
                    od = n[40 * p + 16:40 * p + 40] * rden[2 * p + 1:2 * p + 2]
                    ot[EB * i + 40 * p:EB * i + 40 * p + 40, rs] = _pair_rows(ev, od)
            return c
        lax.fori_loop(0, S // TM, apply, 0)
        out_proj(woa_ref)

    cscale = (DH ** -0.5) * math.log2(math.e) * RADIX / (XMAX * XMAX)
    NC = S // CH

    def layer_b():
        def proj(t, c):
            rs = pl.ds(pl.multiple_of(t * TM, TM), TM)
            xn = _layernorm(xres[rs, :])
            for g in range(NG):
                xs[g] = xn[:, g * LANE:(g + 1) * LANE]
            xp = jnp.concatenate(
                [jnp.concatenate([xs[g, pl.ds(b, LANE, stride=4), :] for g in range(NG)], axis=1)
                 for b in range(4)], axis=0).astype(BF16)
            kt = lax.dot_general(wbt[2 * D:3 * D, :], xp, _NT, preferred_element_type=F32)
            qv = lax.dot_general(wbt[0:2 * D, :], xn.astype(BF16), _NT, preferred_element_type=F32)
            vt[0:D, rs] = qv[D:2 * D]
            for p in range(H // 2):
                (at, tt, bb, mm), me, mo = _limbs(qv[40 * p:40 * p + 40])
                qw[40 * p:40 * p + 40, rs] = _pack4([at, tt, bb, mm])
                cq_s[2 * p:2 * p + 1, rs] = me * cscale
                cq_s[2 * p + 1:2 * p + 2, rs] = mo * cscale
                (at, tt, bb, mm), me, mo = _limbs(kt[40 * p:40 * p + 40])
                for sl, lim in enumerate((at, bb, tt, mm)):
                    ki[pl.ds(160 * p + sl, 40, stride=4), :] = _pack4(
                        [lim[:, b * LANE:(b + 1) * LANE] for b in range(4)])
                cks[2 * p:2 * p + 1, :] = me
                cks[2 * p + 1:2 * p + 2, :] = mo
                ws = pl.ds(pl.multiple_of(t * LANE, LANE), LANE)
                z = lambda n: jnp.zeros((n, LANE), I32)
                k8[2 * p, ws, :] = jnp.concatenate([ki[160 * p:160 * p + 80, :], z(48)], axis=0).T
                k8[2 * p + 1, ws, :] = jnp.concatenate(
                    [z(16), ki[160 * p + 80:160 * p + 160, :], z(32)], axis=0).T
            for b in range(4):
                ckc[t, pl.ds(b, LANE, stride=4), :] = cks[:, b * LANE:(b + 1) * LANE].T
            return c
        lax.fori_loop(0, S // TM, proj, 0)

        def scores(p, odd, t, c):
            h = 2 * p + odd
            qs = pl.ds(pl.multiple_of(t * TQ, TQ), TQ)
            kk = pltpu.bitcast(k8[h, c * (CH // 4):(c + 1) * (CH // 4), :], I8)
            qq = pltpu.bitcast(qw[pl.ds(pl.multiple_of(40 * p + 16 * odd, 8), 32), qs], I8)
            s = jnp.dot(kk, qq, preferred_element_type=I32)
            r0 = (c * CH) % TM
            ck = ckc[(c * CH) // TM, r0:r0 + CH, :]
            ck = jnp.take_along_axis(ck, jnp.full(ck.shape, h, I32), axis=1)
            s = s.astype(F32) * jnp.concatenate([ck] * (TQ // LANE), axis=1)
            sbuf[odd, c * CH:(c + 1) * CH, :] = s
            return jnp.max(s.reshape(CH // 8, 8, TQ), axis=0)

        def pv(p, odd, m, cq, c):
            row = lax.broadcasted_iota(I32, (24, CH), 0)
            pr = jnp.exp2((sbuf[odd, c * CH:(c + 1) * CH, :] - m) * cq)
            v = vt[pl.ds(pl.multiple_of(40 * p + 16 * odd, 8), 24), c * CH:(c + 1) * CH]
            v = jnp.where(row == (0 if odd else 20), 1.0, v)
            return jnp.dot(v, pr, preferred_element_type=F32)

        def mx(a, b):
            return b if a is None else jnp.maximum(a, b)

        mp = None
        for c in range(NC):
            mp = mx(mp, scores(0, 0, 0, c))
        m0 = jnp.max(mp, axis=0, keepdims=True)
        mp1 = None
        for c in range(SK):
            mp1 = mx(mp1, scores(0, 1, 0, c))

        n_units = (H // 2) * NQT

        def body(i, carry):
            m_e, mp_o = carry
            p = i // NQT
            t = i % NQT
            nx = jnp.minimum(i + 1, n_units - 1)
            pn = nx // NQT
            tn = nx % NQT
            qs = pl.ds(pl.multiple_of(t * TQ, TQ), TQ)
            cqe = cq_s[pl.ds(2 * p, 1), qs]
            cqo = cq_s[pl.ds(2 * p + 1, 1), qs]
            acc_e = acc_o = mp_ne = mp_no = m_o = None
            for j in range(2 * NC):
                if j < NC:
                    d = pv(p, 0, m_e, cqe, j)
                    acc_e = d if acc_e is None else acc_e + d
                else:
                    if m_o is None:
                        m_o = jnp.max(mp_o, axis=0, keepdims=True)
                    d = pv(p, 1, m_o, cqo, j - NC)
                    acc_o = d if acc_o is None else acc_o + d
                q = j + SK
                if q < NC:
                    mp_o = mx(mp_o, scores(p, 1, t, q))
                elif q < 2 * NC:
                    mp_ne = mx(mp_ne, scores(pn, 0, tn, q - NC))
                else:
                    mp_no = mx(mp_no, scores(pn, 1, tn, q - 2 * NC))
            oe = acc_e * (1.0 / acc_e[20:21])
            oo = acc_o * (1.0 / acc_o[0:1])
            ot[pl.ds(pl.multiple_of(40 * p, 8), 40), qs] = _pair_rows(oe, oo)
            return jnp.max(mp_ne, axis=0, keepdims=True), mp_no
        lax.fori_loop(0, n_units, body, (m0, mp1))
        out_proj(wob_ref)

    def rep(_, c):
        layer_a()
        layer_b()
        return c
    lax.fori_loop(0, 2, rep, 0)

    o_ref[...] = xres[...].astype(o_ref.dtype)


@jax.jit
def pallas_interleave_layers__linear_attn_block__mha_block__prompt_kernel(
    A_x: jax.Array,
    A_wqkv: jax.Array,
    A_wo: jax.Array,
    B_x: jax.Array,
    B_wqkv: jax.Array,
    B_wo: jax.Array,
):
    del B_x
    x = A_x.reshape(S, D)
    out = pl.pallas_call(
        _kernel,
        out_shape=jax.ShapeDtypeStruct((S, D), A_x.dtype),
        scratch_shapes=[
            pltpu.VMEM((S, D), F32),
            pltpu.VMEM((D, D), BF16),
            pltpu.VMEM((3 * D, D), BF16),
            pltpu.VMEM((H, S // 4, LANE), I32),
            pltpu.VMEM((D + 8, S), I32),
            pltpu.VMEM((4 * D, LANE), I32),
            pltpu.VMEM((NG, TM, LANE), F32),
            pltpu.VMEM((H, S), F32),
            pltpu.VMEM((LANE, TM), F32),
            pltpu.VMEM((S // TM, TM, LANE), F32),
            pltpu.VMEM((D + 8, S), F32),
            pltpu.VMEM((D, S), F32),
            pltpu.VMEM((2, S, TQ), F32),
            pltpu.VMEM((S, D), BF16),
            pltpu.VMEM((S, D), BF16),
            pltpu.VMEM((4, EB + 8, 2 * LANE), BF16),
        ],
        compiler_params=pltpu.CompilerParams(vmem_limit_bytes=110 * 1024 * 1024),
    )(x, A_wqkv, A_wo, B_wqkv, B_wo)
    return out.reshape(A_x.shape)
```

```python
import math

import jax
import jax.numpy as jnp
from jax import lax
import jax.experimental.pallas as pl
import jax.experimental.pallas.tpu as pltpu

S = 2048
D = 640
H = 32
DH = 20
LANE = 128
NG = D // LANE
TM = 512
HM = TM // 2
NT_ = S // TM
TQ = 512
CH = 128
NQT = S // TQ
UNROLL = 1
NC = S // CH
RB = 160
EB = 160

F32 = jnp.float32
BF16 = jnp.bfloat16
I32 = jnp.int32
I8 = jnp.int8

NCOPY = 3
MAGIC = 1.5 * 2.0 ** 23
CSCALE = (DH ** -0.5) * math.log2(math.e) / NCOPY

_NT = (((1,), (1,)), ((), ()))
_TN = (((0,), (0,)), ((), ()))


def _layernorm(x):
    m = jnp.mean(x, axis=-1, keepdims=True)
    xc = x - m
    v = jnp.mean(xc * xc, axis=-1, keepdims=True)
    return xc * lax.rsqrt(v + 1e-5)


def _phi(t):
    return jnp.where(t > 0, t + 1.0, jnp.exp(t)) + 1e-6


def _pair_rows(even, odd):
    n = even.shape[1]
    row = lax.broadcasted_iota(I32, (8, n), 0)
    mid = jnp.where(row < 4, even[16:24], odd[0:8])
    return jnp.concatenate([even[0:16], mid, odd[8:24]], axis=0)


def _pair_absmax(a):
    lo = lax.broadcasted_iota(I32, (8, a.shape[1]), 0) < 4
    me = jnp.maximum(jnp.maximum(a[0:8], a[8:16]), jnp.where(lo, a[16:24], 0.0))
    mo = jnp.maximum(jnp.maximum(a[24:32], a[32:40]), jnp.where(lo, 0.0, a[16:24]))
    return jnp.max(me, axis=0, keepdims=True), jnp.max(mo, axis=0, keepdims=True)


def _pair_scale(blk, se, so):
    lo = lax.broadcasted_iota(I32, (8, blk.shape[1]), 0) < 4
    return jnp.concatenate(
        [blk[0:16] * se, blk[16:24] * jnp.where(lo, se, so), blk[24:40] * so], axis=0)


def _limbs(u16):
    x = pltpu.bitcast(u16 + (MAGIC + 8.0), I32)
    return x >> 4, pltpu.bitcast(u16 * (NCOPY / 256.0) + MAGIC, I32), x


def _pack4(xs):
    return pltpu.bitcast(pltpu.pack_elementwise(xs, packed_dtype=I8), I32)


def _transposed(w_ref, col):
    return _pack2(w_ref[:, col:col + LANE].astype(F32).T)


def _pack2(x):
    return pltpu.bitcast(x.astype(BF16), I32)


def _unpack(ref, r0=0, n=None):
    n = 2 * ref.shape[0] if n is None else n
    if isinstance(r0, int):
        return pltpu.bitcast(ref[r0 // 2:(r0 + n) // 2, :], BF16)
    return pltpu.bitcast(ref[pl.ds(pl.multiple_of(r0 // 2, 8), n // 2), :], BF16)


def _kernel(x_hbm, wa_hbm, woa_hbm, wb_hbm, wob_hbm, o_hbm,
            xio, wa, woa, wb, wob, xres, wat, wbt, k8, qw, q5, ki, xs, xnb, kraw, kam, sk_s, qf_s, mg_s, vt, ot, sbuf,
            g_s, z_s, rd_s, m_s, zb, xsem, wsem, osem):
    def tile(t, n=TM, off=0):
        return pl.ds(pl.multiple_of(t * TM + off, LANE), n)

    def x_copy(t):
        return pltpu.make_async_copy(x_hbm.at[tile(t)], xio.at[tile(t)], xsem.at[t])

    def o_copy(t):
        return pltpu.make_async_copy(xio.at[tile(t)], o_hbm.at[tile(t)], osem.at[t])

    w_copies = [pltpu.make_async_copy(src, dst, wsem.at[i]) for i, (src, dst) in enumerate(
        ((wa_hbm, wa), (woa_hbm, woa), (wb_hbm, wb), (wob_hbm, wob)))]

    w_copies[0].start()
    for t in range(NT_):
        x_copy(t).start()
    for c in w_copies[1:]:
        c.start()
    kam[...] = jnp.zeros(kam.shape, F32)
    zb[...] = jnp.zeros(zb.shape, F32)
    g_s[...] = jnp.zeros(g_s.shape, F32)
    z_s[...] = jnp.zeros(z_s.shape, F32)
    w_copies[0].wait()
    for j in range(2 * NG):
        wat[j * 64:(j + 1) * 64, :] = _transposed(wa, j * LANE)

    def proj_a(t, halves):
        xn = [_layernorm(x).astype(BF16) for x in halves]
        pk = []
        for i in range(2):
            pk.append(_phi(lax.dot_general(_unpack(wat, D, D), xn[i], _NT, preferred_element_type=F32)))
        for i in range(2):
            q = lax.dot_general(_unpack(wat, 0, D), xn[i], _NT, preferred_element_type=F32)
            ot[:, tile(t, HM, i * HM)] = _phi(q)
        pkf = jnp.concatenate(pk, axis=1)
        g_s[...] += jnp.dot(pkf.astype(BF16), jnp.concatenate(xn, axis=0), preferred_element_type=F32)
        zp = pkf[:, 0:LANE]
        for j in range(1, TM // LANE):
            zp = zp + pkf[:, j * LANE:(j + 1) * LANE]
        z_s[...] += zp

    def mid_a():
        z = jnp.sum(z_s[...].T, axis=0, keepdims=True)
        hd = lax.broadcasted_iota(I32, (H, D), 0) * DH
        d = lax.broadcasted_iota(I32, (H, D), 1)
        zt = jnp.where(jnp.logical_and(d >= hd, d < hd + DH), z, 0.0)
        for t in range(NT_):
            den = jnp.dot(zt, ot[:, t * TM:(t + 1) * TM], preferred_element_type=F32)
            rd_s[:, t * TM:(t + 1) * TM] = 1.0 / (den + 1e-6)
        z_s[...] = jnp.zeros(z_s.shape, F32)
        for i in range(4):
            kv = jnp.dot(g_s[EB * i:EB * (i + 1), :].astype(BF16),
                         wa[:, 2 * D + LANE * i:2 * D + LANE * i + 2 * LANE],
                         preferred_element_type=F32)
            r = lax.broadcasted_iota(I32, kv.shape, 0)
            e = lax.broadcasted_iota(I32, kv.shape, 1) + (LANE * i - EB * i)
            hr = (r // DH) * DH
            keep = jnp.logical_and(e >= hr, e < hr + DH)
            kv = jnp.where(keep, kv, 0.0).astype(BF16)
            m_s[EB // 2 * i:EB // 2 * (i + 1), :] = _pack2(jnp.dot(
                kv, woa[LANE * i:LANE * i + 2 * LANE, :], preferred_element_type=F32))
        g_s[...] = jnp.zeros(g_s.shape, F32)
        for j in range(3 * NG):
            wbt[j * 64:(j + 1) * 64, :] = _transposed(wb, j * LANE)

    def out_a(t, i):
        rs = tile(t, HM, i * HM)
        r = rd_s[:, rs]
        pqn = jnp.concatenate(
            [_pair_scale(ot[40 * p:40 * p + 40, rs], r[2 * p:2 * p + 1], r[2 * p + 1:2 * p + 2])
             for p in range(H // 2)], axis=0)
        x = xres[rs, :] + lax.dot_general(pqn, _unpack(m_s), _TN, preferred_element_type=F32)
        xres[rs, :] = x
        return x

    def proj_b1(t):
        xn = [_layernorm(out_a(t, i)) for i in range(2)]
        for i in range(2):
            for g in range(NG):
                xs[g, i * HM:(i + 1) * HM, :] = xn[i][:, g * LANE:(g + 1) * LANE]
        for i in range(2):
            rs = tile(t, HM, i * HM)
            xb = xn[i].astype(BF16)
            xnb[pl.ds(pl.multiple_of((t * TM + i * HM) // 2, 8), HM // 2), :] = pltpu.bitcast(xb, I32)
            vt[:, rs] = lax.dot_general(_unpack(wbt, 0, D), xb, _NT, preferred_element_type=F32)
        xp = jnp.concatenate(
            [jnp.concatenate([xs[g, pl.ds(b, LANE, stride=4), :] for g in range(NG)], axis=1)
             for b in range(4)], axis=0).astype(BF16)
        kt = lax.dot_general(_unpack(wbt, D, D), xp, _NT, preferred_element_type=F32)
        kraw[:, tile(t)] = kt
        a = kam[...]
        for b in range(4):
            a = jnp.maximum(a, jnp.abs(kt[:, b * LANE:(b + 1) * LANE]))
        kam[...] = a

    def mid_b():
        for p in range(H // 2):
            me, mo = _pair_absmax(kam[40 * p:40 * p + 40, :])
            me = jnp.maximum(jnp.max(me, axis=1, keepdims=True), 1e-30)
            mo = jnp.maximum(jnp.max(mo, axis=1, keepdims=True), 1e-30)
            sk_s[40 * p:40 * p + 40, :] = _pair_scale(jnp.full((40, LANE), 16.0 * 127.0, F32), 1.0 / me, 1.0 / mo)
            qf_s[2 * p:2 * p + 1, :] = jnp.broadcast_to(me * (CSCALE / 127.0), (1, LANE))
            qf_s[2 * p + 1:2 * p + 2, :] = jnp.broadcast_to(mo * (CSCALE / 127.0), (1, LANE))
        kam[...] = jnp.zeros(kam.shape, F32)

    def proj_b2(t):
        rs = tile(t)
        ws = pl.ds(pl.multiple_of(t * LANE, LANE), LANE)
        z8 = jnp.zeros((8, TM), I32)
        lo = lax.broadcasted_iota(I32, (8, LANE), 0) < 4
        z = lambda n: jnp.zeros((n, LANE), I32)
        for p in range(H // 2):
            q = vt[40 * p:40 * p + 40, rs]
            sc = []
            for odd, am in enumerate(_pair_absmax(jnp.abs(q))):
                qf = qf_s[2 * p + odd:2 * p + odd + 1, :]
                qf = jnp.concatenate([qf] * (TM // LANE), axis=1)
                w = jnp.clip(am * (qf * (1.0 / 127.0)), 2.0 ** -100, 2.0 ** 100)
                unit = (pltpu.bitcast(w, I32) + 0x007FFFFF) & 0x7F800000
                mg_s[2 * p + odd:2 * p + odd + 1, rs] = unit + ((23 << 23) + 0x00400000)
                sc.append((qf * 16.0) * pltpu.bitcast(0x7F000000 - unit, F32))
            hi, tt, ll = _limbs(_pair_scale(q, *sc))
            qw[40 * p:40 * p + 40, rs] = (_pack4([hi, hi, tt, ll]) & 0x0FFFFFFF) - (8 << 24)
            for odd in range(2):
                win = jnp.concatenate([hi[16 * odd:16 * odd + 24], z8], axis=0).astype(I8)
                q5[16 * p + 8 * odd:16 * p + 8 * odd + 8, rs] = pltpu.bitcast(win, I32)

            sk = sk_s[40 * p:40 * p + 40, :]
            lims = [_limbs(kraw[40 * p:40 * p + 40, tile(t, LANE, b * LANE)] * sk) for b in range(4)]
            hi, tt, ll = [_pack4([lims[b][j] for b in range(4)]) for j in range(3)]
            ll = ((ll & 0x0F0F0F0F) + 0x78787878) ^ (0x80808080 - (1 << 32))
            for sl, w in enumerate((hi, hi, ll, tt)):
                ki[pl.ds(160 * p + sl, 40, stride=4), :] = w
            k8[2 * p, ws, :] = jnp.concatenate(
                [ki[160 * p:160 * p + 80, :], z(16),
                 hi[0:16], jnp.where(lo, hi[16:24], 0), z(8)], axis=0).T
            k8[2 * p + 1, ws, :] = jnp.concatenate(
                [z(16), ki[160 * p + 80:160 * p + 160, :],
                 jnp.where(lo, 0, hi[16:24]), hi[24:40], z(8)], axis=0).T
            if p % (RB // 40) == RB // 40 - 1:
                r0 = 40 * (p + 1) - RB
                v = lax.dot_general(
                    _unpack(wbt, 2 * D + r0, RB), _unpack(xnb, t * TM, TM), _NT, preferred_element_type=F32)
                vt[r0:r0 + RB, rs] = v
                kraw[r0:r0 + RB, rs] = v

    def scores(p, odd, t, mg, c):
        h = 2 * p + odd
        qs = pl.ds(pl.multiple_of(t * TQ, TQ), TQ)
        kk = pltpu.bitcast(k8[h, c * (CH // 4):(c + 1) * (CH // 4), :], I8)
        qq = jnp.concatenate([qw[pl.ds(pl.multiple_of(40 * p + 16 * odd, 8), 24), qs],
                              q5[pl.ds(pl.multiple_of(8 * h, 8), 8), qs]], axis=0)
        s = jnp.dot(kk, pltpu.bitcast(qq, I8), preferred_element_type=I32)
        return pltpu.bitcast(s + mg, F32)

    def keep(s, odd, c, mp):
        sbuf[odd, c * CH:(c + 1) * CH, :] = s
        mc = jnp.max(s.reshape(CH // 8, 8, TQ), axis=0)
        return mc if mp is None else jnp.maximum(mp, mc)

    def magic(p, odd, t):
        return mg_s[pl.ds(2 * p + odd, 1), pl.ds(pl.multiple_of(t * TQ, TQ), TQ)]

    def pv(p, odd, m, c):
        row = lax.broadcasted_iota(I32, (24, CH), 0)
        pr = jnp.exp2(sbuf[odd, c * CH:(c + 1) * CH, :] - m)
        v = vt[pl.ds(pl.multiple_of(40 * p + 16 * odd, 8), 24), c * CH:(c + 1) * CH]
        v = jnp.where(row == (0 if odd else 20), 1.0, v)
        return jnp.dot(v, pr, preferred_element_type=F32)

    def attention():
        m0 = []
        for odd in range(2):
            mp = None
            mg = magic(0, odd, 0)
            for c in range(NC):
                mp = keep(scores(0, odd, 0, mg, c), odd, c, mp)
            m0.append(mp)

        n_units = (H // 2) * NQT

        def unit(i, carry):
            p = i // NQT
            t = i % NQT
            nx = jnp.minimum(i + 1, n_units - 1)
            pn = nx // NQT
            tn = nx % NQT
            outs, mps = [], []
            for odd in range(2):
                m = jnp.max(carry[odd], axis=0, keepdims=True)
                mg = magic(pn, odd, tn)
                acc = zb[...]
                mp = None
                for c in range(NC):
                    s = scores(pn, odd, tn, mg, c)
                    acc = acc + pv(p, odd, m, c)
                    mp = keep(s, odd, c, mp)
                r = 0 if odd else 20
                outs.append(acc * (1.0 / acc[r:r + 1]))
                mps.append(mp)
            qs = pl.ds(pl.multiple_of(t * TQ, TQ), TQ)
            ot[pl.ds(pl.multiple_of(40 * p, 8), 40), qs] = _pair_rows(*outs)
            return tuple(mps)

        def body(i, carry):
            for u in range(UNROLL):
                carry = unit(UNROLL * i + u, carry)
            return carry
        lax.fori_loop(0, n_units // UNROLL, body, tuple(m0))

    def out_b(t, i):
        rs = tile(t, HM, i * HM)
        return xres[rs, :] + lax.dot_general(ot[:, rs], wob[...], _TN, preferred_element_type=F32)

    def first(t, c):
        x_copy(t).wait()
        halves = []
        for i in range(2):
            rs = tile(t, HM, i * HM)
            x = xio[rs, :].astype(F32)
            xres[rs, :] = x
            halves.append(x)
        proj_a(t, halves)
        return c
    lax.fori_loop(0, NT_, first, 0)
    for c in w_copies[1:]:
        c.wait()

    def rep(r, carry):
        mid_a()

        def b1(t, c):
            proj_b1(t)
            return c
        lax.fori_loop(0, NT_, b1, 0)
        mid_b()

        def b2(t, c):
            proj_b2(t)
            return c
        lax.fori_loop(0, NT_, b2, 0)
        attention()

        @pl.when(r == 0)
        def _():
            def b_to_a(t, c):
                halves = [out_b(t, 0), out_b(t, 1)]
                for i in range(2):
                    xres[tile(t, HM, i * HM), :] = halves[i]
                proj_a(t, halves)
                return c
            lax.fori_loop(0, NT_, b_to_a, 0)

        @pl.when(r == 1)
        def _():
            def last(t, c):
                for i in range(2):
                    xio[tile(t, HM, i * HM), :] = out_b(t, i).astype(xio.dtype)
                o_copy(t).start()
                return c
            lax.fori_loop(0, NT_, last, 0)
        return carry
    lax.fori_loop(0, 2, rep, 0)
    for t in range(NT_):
        o_copy(t).wait()


@jax.jit
def pallas_interleave_layers__linear_attn_block__mha_block__prompt_kernel(
    A_x: jax.Array,
    A_wqkv: jax.Array,
    A_wo: jax.Array,
    B_x: jax.Array,
    B_wqkv: jax.Array,
    B_wo: jax.Array,
):
    del B_x
    x = A_x.reshape(S, D)
    out = pl.pallas_call(
        _kernel,
        out_shape=jax.ShapeDtypeStruct((S, D), A_x.dtype),
        in_specs=[pl.BlockSpec(memory_space=pl.ANY)] * 5,
        out_specs=pl.BlockSpec(memory_space=pl.ANY),
        scratch_shapes=[
            pltpu.VMEM((S, D), BF16),
            pltpu.VMEM((D, 3 * D), BF16),
            pltpu.VMEM((D, D), BF16),
            pltpu.VMEM((D, 3 * D), BF16),
            pltpu.VMEM((D, D), BF16),
            pltpu.VMEM((S, D), F32),
            pltpu.VMEM((D, D), I32),
            pltpu.VMEM((3 * D // 2, D), I32),
            pltpu.VMEM((H, S // 4, LANE), I32),
            pltpu.VMEM((D, S), I32),
            pltpu.VMEM((8 * H, S), I32),
            pltpu.VMEM((4 * D, LANE), I32),
            pltpu.VMEM((NG, TM, LANE), F32),
            pltpu.VMEM((S // 2, D), I32),
            pltpu.VMEM((D, S), F32),
            pltpu.VMEM((D, LANE), F32),
            pltpu.VMEM((D, LANE), F32),
            pltpu.VMEM((H, LANE), F32),
            pltpu.VMEM((H, S), I32),
            pltpu.VMEM((D, S), F32),
            pltpu.VMEM((D, S), F32),
            pltpu.VMEM((2, S, TQ), F32),
            pltpu.VMEM((D, D), F32),
            pltpu.VMEM((D, LANE), F32),
            pltpu.VMEM((H, S), F32),
            pltpu.VMEM((D // 2, D), I32),
            pltpu.VMEM((24, TQ), F32),
            pltpu.SemaphoreType.DMA((NT_,)),
            pltpu.SemaphoreType.DMA((4,)),
            pltpu.SemaphoreType.DMA((NT_,)),
        ],
        compiler_params=pltpu.CompilerParams(vmem_limit_bytes=110 * 1024 * 1024),
    )(x, A_wqkv, A_wo, B_wqkv, B_wo)
    return out.reshape(A_x.shape)
```

```python
import math

import jax
import jax.numpy as jnp
from jax import lax
import jax.experimental.pallas as pl
import jax.experimental.pallas.tpu as pltpu

S = 2048
D = 640
H = 32
DH = 20
LANE = 128
NG = D // LANE
TM = 512
HM = TM // 2
NT_ = S // TM
TQ = 512
CH = 128
NQT = S // TQ
NC = S // CH
UNROLL = 2
RB = 160
OB = 64
EVERY = 2 * UNROLL * NC * OB // S

F32 = jnp.float32
BF16 = jnp.bfloat16
I32 = jnp.int32
I8 = jnp.int8

NCOPY = 3
UMAX = 126.5
BIG = 3e38
MAGIC = 1.5 * 2.0 ** 23
CSCALE = (DH ** -0.5) * math.log2(math.e) / NCOPY

_NT = (((1,), (1,)), ((), ()))
_TN = (((0,), (0,)), ((), ()))


def _layernorm(x):
    m = jnp.mean(x, axis=-1, keepdims=True)
    xc = x - m
    v = jnp.mean(xc * xc, axis=-1, keepdims=True)
    return xc * lax.rsqrt(v + 1e-5)


def _phi(t):
    return jnp.where(t > 0, t + 1.0, jnp.exp(t)) + 1e-6


def _pair_rows(even, odd):
    n = even.shape[1]
    row = lax.broadcasted_iota(I32, (8, n), 0)
    mid = jnp.where(row < 4, even[16:24], odd[0:8])
    return jnp.concatenate([even[0:16], mid, odd[8:24]], axis=0)


def _pair_absmax(a):
    lo = lax.broadcasted_iota(I32, (8, a.shape[1]), 0) < 4
    me = jnp.maximum(jnp.maximum(a[0:8], a[8:16]), jnp.where(lo, a[16:24], 0.0))
    mo = jnp.maximum(jnp.maximum(a[24:32], a[32:40]), jnp.where(lo, 0.0, a[16:24]))
    return jnp.max(me, axis=0, keepdims=True), jnp.max(mo, axis=0, keepdims=True)


def _pair_scale(blk, se, so):
    lo = lax.broadcasted_iota(I32, (8, blk.shape[1]), 0) < 4
    return jnp.concatenate(
        [blk[0:16] * se, blk[16:24] * jnp.where(lo, se, so), blk[24:40] * so], axis=0)


def _i32(v):
    return v - (1 << 32) if v >= (1 << 31) else v


def _pack_key_limbs(x, t):
    x = [pltpu.bitcast(v, I32) for v in x]
    t = [pltpu.bitcast(v, I32) for v in t]
    w02 = x[0] + (x[2] << 16)
    w13 = x[1] + (x[3] << 16)
    flip = _i32(0x80808080)
    hi = (((w02 >> 4) & 0x00FF00FF) | ((w13 << 4) & _i32(0xFF00FF00))) ^ flip
    ll = (((w02 & 0x000F000F) | ((w13 << 8) & 0x0F000F00)) + 0x78787878) ^ flip
    tt = (((t[0] + (t[1] << 8)) + ((t[2] << 16) + (t[3] << 24))) - 0x50000000) ^ flip
    return hi, tt, ll


def _transposed(w_ref, col):
    return _pack2(w_ref[:, col:col + LANE].astype(F32).T)


def _pack2(x):
    return pltpu.bitcast(x.astype(BF16), I32)


def _unpack(ref, r0=0, n=None):
    n = 2 * ref.shape[0] if n is None else n
    if isinstance(r0, int):
        return pltpu.bitcast(ref[r0 // 2:(r0 + n) // 2, :], BF16)
    return pltpu.bitcast(ref[pl.ds(pl.multiple_of(r0 // 2, 8), n // 2), :], BF16)


def _kernel(x_hbm, wa_hbm, woa_hbm, wb_hbm, wob_hbm, o_hbm,
            xio, wa, woa, wb, wob, xres, wat, wbt, k8, qw, xs, xnb, kraw, kmm, ks_s, mg_s, vt, ot, sbuf,
            g_s, z_s, rd_s, m_s, zb, xsem, wsem, osem):
    def tile(t, n=TM, off=0):
        return pl.ds(pl.multiple_of(t * TM + off, LANE), n)

    def x_copy(t):
        return pltpu.make_async_copy(x_hbm.at[tile(t)], xio.at[tile(t)], xsem.at[t])

    def o_copy(t, i):
        rs = tile(t, HM, i * HM)
        return pltpu.make_async_copy(xio.at[rs], o_hbm.at[rs], osem.at[2 * t + i])

    def wa_copy(j):
        cs = pl.ds(j * D, D)
        return pltpu.make_async_copy(wa_hbm.at[:, cs], wa.at[:, cs], wsem.at[j])

    w_copies = [wa_copy(2)] + [
        pltpu.make_async_copy(src, dst, wsem.at[3 + i]) for i, (src, dst) in enumerate(
            ((woa_hbm, woa), (wb_hbm, wb), (wob_hbm, wob)))]

    wa_copy(0).start()
    wa_copy(1).start()
    for t in range(NT_):
        x_copy(t).start()
    for c in w_copies:
        c.start()
    zb[...] = jnp.zeros(zb.shape, F32)
    xs[:, TM:TM + 32, :] = jnp.zeros((NG, 32, LANE), F32)
    g_s[...] = jnp.zeros(g_s.shape, F32)
    z_s[...] = jnp.zeros(z_s.shape, F32)
    for part in range(2):
        wa_copy(part).wait()
        for j in range(part * NG, (part + 1) * NG):
            wat[j * 64:(j + 1) * 64, :] = _transposed(wa, j * LANE)

    def proj_a(t, parts):
        xn = [_layernorm(x).astype(BF16) for x in parts]
        pk = []
        for x in xn:
            pk.append(_phi(lax.dot_general(_unpack(wat, D, D), x, _NT, preferred_element_type=F32)))
        off = 0
        for x in xn:
            q = lax.dot_general(_unpack(wat, 0, D), x, _NT, preferred_element_type=F32)
            ot[:, tile(t, x.shape[0], off)] = _phi(q)
            off += x.shape[0]
        pkf = jnp.concatenate(pk, axis=1)
        g_s[...] += jnp.dot(pkf.astype(BF16), jnp.concatenate(xn, axis=0), preferred_element_type=F32)
        zp = pkf[:, 0:LANE]
        for j in range(1, TM // LANE):
            zp = zp + pkf[:, j * LANE:(j + 1) * LANE]
        z_s[...] += zp

    def mid_a():
        lo = [(LANE * j // DH) * DH // 16 * 16 for j in range(NG)] + [D]
        hi = [-(-((LANE * j + LANE - 1) // DH + 1) * DH // 16) * 16 for j in range(NG)]
        kvs = []
        for j in range(NG):
            kv = jnp.dot(g_s[lo[j]:hi[j], :].astype(BF16),
                         wa[:, 2 * D + LANE * j:2 * D + LANE * (j + 1)], preferred_element_type=F32)
            he = (lax.broadcasted_iota(I32, (1, LANE), 1) + LANE * j) // DH * DH - lo[j]
            r = lax.broadcasted_iota(I32, kv.shape, 0)
            kvs.append(jnp.where(jnp.logical_and(r >= he, r < he + DH), kv, 0.0).astype(BF16))
        z = jnp.sum(z_s[...].T, axis=0, keepdims=True)
        hd = lax.broadcasted_iota(I32, (H, D), 0) * DH
        d = lax.broadcasted_iota(I32, (H, D), 1)
        zt = jnp.where(jnp.logical_and(d >= hd, d < hd + DH), z, 0.0)
        for t in range(NT_):
            den = jnp.dot(zt, ot[:, t * TM:(t + 1) * TM], preferred_element_type=F32)
            rd_s[:, t * TM:(t + 1) * TM] = 1.0 / (den + 1e-6)
        z_s[...] = jnp.zeros(z_s.shape, F32)
        prev = None
        for j in range(NG):
            m = jnp.dot(kvs[j], woa[LANE * j:LANE * (j + 1), :], preferred_element_type=F32)
            r0 = lo[j]
            if prev is not None:
                n = hi[j - 1] - r0
                m_s[r0 // 2:hi[j - 1] // 2, :] = _pack2(prev + m[0:n])
                m, r0 = m[n:], hi[j - 1]
            m_s[r0 // 2:lo[j + 1] // 2, :] = _pack2(m[0:lo[j + 1] - r0])
            prev = m[lo[j + 1] - r0:] if j + 1 < NG else None
        g_s[...] = jnp.zeros(g_s.shape, F32)
        for j in range(3 * NG):
            wbt[j * 64:(j + 1) * 64, :] = _transposed(wb, j * LANE)

    def out_a(t, i):
        rs = tile(t, HM, i * HM)
        r = rd_s[:, rs]
        pqn = jnp.concatenate(
            [_pair_scale(ot[40 * p:40 * p + 40, rs], r[2 * p:2 * p + 1], r[2 * p + 1:2 * p + 2])
             for p in range(H // 2)], axis=0)
        x = xres[rs, :] + lax.dot_general(pqn, _unpack(m_s), _TN, preferred_element_type=F32)
        xres[rs, :] = x
        return x

    def proj_b1(t):
        xn = [_layernorm(out_a(t, i)) for i in range(2)]
        for i in range(2):
            for g in range(NG):
                xs[g, i * HM:(i + 1) * HM, :] = xn[i][:, g * LANE:(g + 1) * LANE]
        for i in range(2):
            rs = tile(t, HM, i * HM)
            xb = xn[i].astype(BF16)
            xnb[pl.ds(pl.multiple_of((t * TM + i * HM) // 2, 8), HM // 2), :] = pltpu.bitcast(xb, I32)
            if i == 0:
                vt[:, rs] = lax.dot_general(_unpack(wbt, 2 * D, D), xb, _NT, preferred_element_type=F32)
        xp = jnp.concatenate(
            [jnp.concatenate([xs[g, pl.ds(b, LANE, stride=4), :] for g in range(NG)], axis=1)
             for b in range(4)], axis=0).astype(BF16)
        kt = lax.dot_general(_unpack(wbt, D, D), xp, _NT, preferred_element_type=F32)
        kraw[:, tile(t)] = kt
        hi, lo = kmm[0], kmm[1]
        for b in range(4):
            hi = jnp.maximum(hi, kt[:, b * LANE:(b + 1) * LANE])
            lo = jnp.minimum(lo, kt[:, b * LANE:(b + 1) * LANE])
        kmm[0] = hi
        kmm[1] = lo

    def reset_kmm():
        kmm[0] = jnp.full((D, LANE), -BIG, F32)
        kmm[1] = jnp.full((D, LANE), BIG, F32)

    def mid_b():
        hi = jnp.max(kmm[0], axis=1, keepdims=True)
        lo = jnp.min(kmm[1], axis=1, keepdims=True)
        ce = 0.5 * hi + 0.5 * lo
        hr = jnp.maximum(jnp.maximum(0.5 * hi - 0.5 * lo, jnp.abs(ce) * 2.0 ** -11), 1e-30)
        sk = (1024.0 * 16.0 * UMAX) / hr
        for j, v in enumerate((sk, (2.0 ** 33 + 1024.0 * 2056.0) - ce * sk,
                               sk * (NCOPY / 256.0),
                               (2.0 ** 33 + 1024.0 * 128.0) - ce * sk * (NCOPY / 256.0),
                               hr * (CSCALE / UMAX))):
            ks_s[j] = jnp.broadcast_to(v, (D, LANE))
        reset_kmm()

    def proj_b2(t):
        rs = tile(t)
        ws = pl.ds(pl.multiple_of(t * LANE, LANE), LANE)
        z8 = jnp.zeros((8, TM), I32)
        lo = lax.broadcasted_iota(I32, (8, LANE), 0) < 4
        for p in range(H // 2):
            pr = slice(40 * p, 40 * p + 40)
            if p % (RB // 40) == 0:
                qb = lax.dot_general(_unpack(wbt, 40 * p, RB), _unpack(xnb, t * TM, TM), _NT,
                                     preferred_element_type=F32)
            pp = p % (RB // 40)
            q = qb[40 * pp:40 * pp + 40] * jnp.concatenate([ks_s[4, pr, :]] * (TM // LANE), axis=1)
            sc = []
            for odd, am in enumerate(_pair_absmax(jnp.abs(q))):
                w = jnp.clip(am * (1.0 / 127.0), 2.0 ** -100, 2.0 ** 100)
                unit = (pltpu.bitcast(w, I32) + 0x007FFFFF) & 0x7F800000
                mg_s[2 * p + odd:2 * p + odd + 1, rs] = unit + ((23 << 23) + 0x00400000)
                sc.append(16.0 * pltpu.bitcast(0x7F000000 - unit, F32))
            u16 = _pair_scale(q, *sc)
            x16 = pltpu.bitcast(u16 + (MAGIC + 8.0), I32)
            hi = x16 >> 4
            ll = (x16 & 15) - 8
            tt = pltpu.bitcast(u16 * (NCOPY / 256.0) + MAGIC, I32)
            for odd in range(2):
                w = slice(16 * odd, 16 * odd + 24)
                blk = jnp.concatenate([hi[w], hi[w], hi[w], tt[w], ll[w], z8], axis=0).astype(I8)
                qw[64 * p + 32 * odd:64 * p + 32 * odd + 32, rs] = pltpu.bitcast(blk, I32)

            ks = [kraw[pr, tile(t, LANE, b * LANE)] for b in range(4)]
            hi, tt, ll = _pack_key_limbs([k * ks_s[0, pr, :] + ks_s[1, pr, :] for k in ks],
                                         [k * ks_s[2, pr, :] + ks_s[3, pr, :] for k in ks])
            ev = [[x[0:16], jnp.where(lo, x[16:24], 0)] for x in (hi, ll, tt)]
            od = [[jnp.where(lo, 0, x[16:24]), x[24:40]] for x in (hi, ll, tt)]
            for odd, (h3, l3, t3) in enumerate((ev, od)):
                k8[2 * p + odd, ws, :] = jnp.concatenate(
                    h3 + h3 + h3 + l3 + t3 + [jnp.zeros((8, LANE), I32)], axis=0).T
        vt[:, tile(t, HM, HM)] = lax.dot_general(
            _unpack(wbt, 2 * D, D), _unpack(xnb, t * TM + HM, HM), _NT, preferred_element_type=F32)

    def scores(p, odd, t, mg, c):
        h = 2 * p + odd
        qs = pl.ds(pl.multiple_of(t * TQ, TQ), TQ)
        kk = pltpu.bitcast(k8[h, c * (CH // 4):(c + 1) * (CH // 4), :], I8)
        qq = qw[pl.ds(pl.multiple_of(32 * h, 32), 32), qs]
        s = jnp.dot(kk, pltpu.bitcast(qq, I8), preferred_element_type=I32)
        return pltpu.bitcast(s + mg, F32)

    def keep(s, slot, c, mp):
        sbuf[slot, c * CH:(c + 1) * CH, :] = s
        mc = jnp.max(s.reshape(CH // 8, 8, TQ), axis=0)
        return mc if mp is None else jnp.maximum(mp, mc)

    def magic(p, odd, t):
        return mg_s[pl.ds(2 * p + odd, 1), pl.ds(pl.multiple_of(t * TQ, TQ), TQ)]

    def pv(p, odd, slot, m, c):
        row = lax.broadcasted_iota(I32, (24, CH), 0)
        pr = jnp.exp2(sbuf[slot, c * CH:(c + 1) * CH, :] - m)
        v = vt[pl.ds(pl.multiple_of(40 * p + 16 * odd, 8), 24), c * CH:(c + 1) * CH]
        v = jnp.where(row == (0 if odd else 20), 1.0, v)
        return jnp.dot(v, pr, preferred_element_type=F32)

    def out_b0(j):
        r0 = j * OB
        b0 = r0 // LANE * LANE
        o = ot[0:LANE, b0:b0 + LANE].T[r0 - b0:r0 - b0 + OB]
        xres[r0:r0 + OB, :] += jnp.dot(o.astype(BF16), wob[0:LANE, :], preferred_element_type=F32)

    def attention():
        n_units = (H // 2) * NQT

        def step(i, carry, do_pv=True, do_qk=True):
            mps = []
            for u in range(UNROLL):
                cur = UNROLL * i + u
                nx = cur + UNROLL
                p, t, pn, tn = cur >> 2, cur & 3, nx >> 2, nx & 3
                outs = []
                for odd in range(2):
                    slot = 2 * u + odd
                    if do_pv:
                        m = jnp.max(carry[slot], axis=0, keepdims=True)
                        acc = zb[...]
                    if do_qk:
                        mg = magic(pn, odd, tn)
                    mp = None
                    for c in range(NC):
                        if do_qk:
                            s = scores(pn, odd, tn, mg, c)
                        if do_pv:
                            acc = acc + pv(p, odd, slot, m, c)
                        if do_qk:
                            mp = keep(s, slot, c, mp)
                        elif (slot * NC + c) % EVERY == 0:
                            out_b0((slot * NC + c) // EVERY)
                    if do_pv:
                        r = 0 if odd else 20
                        outs.append(acc * (1.0 / acc[r:r + 1]))
                    mps.append(mp)
                if do_pv:
                    qs = pl.ds(pl.multiple_of(t * TQ, TQ), TQ)
                    ot[pl.ds(pl.multiple_of(40 * p, 8), 40), qs] = _pair_rows(*outs)
            return tuple(mps)

        n_steps = n_units // UNROLL
        carry = step(-1, None, do_pv=False)
        carry = lax.fori_loop(0, n_steps - 1, step, carry)
        step(n_steps - 1, carry, do_qk=False)

    def out_b(t, i):
        rs = tile(t, HM, i * HM)
        return xres[rs, :] + lax.dot_general(
            ot[LANE:D, rs], wob[LANE:D, :], _TN, preferred_element_type=F32)

    reset_kmm()

    def first(t, c):
        x_copy(t).wait()
        halves = []
        for i in range(2):
            rs = tile(t, HM, i * HM)
            x = xio[rs, :].astype(F32)
            xres[rs, :] = x
            halves.append(x)
        proj_a(t, halves)
        return c
    lax.fori_loop(0, NT_, first, 0)
    for c in w_copies:
        c.wait()

    def rep(r, carry):
        mid_a()

        def b1(t, c):
            proj_b1(t)
            return c
        lax.fori_loop(0, NT_, b1, 0)
        mid_b()

        def b2(t, c):
            proj_b2(t)
            return c
        lax.fori_loop(0, NT_, b2, 0)
        attention()

        @pl.when(r == 0)
        def _():
            def b_to_a(t, c):
                halves = [out_b(t, 0), out_b(t, 1)]
                for i in range(2):
                    xres[tile(t, HM, i * HM), :] = halves[i]
                proj_a(t, halves)
                return c
            lax.fori_loop(0, NT_, b_to_a, 0)

        @pl.when(r == 1)
        def _():
            def last(t, c):
                for i in range(2):
                    xio[tile(t, HM, i * HM), :] = out_b(t, i).astype(xio.dtype)
                    o_copy(t, i).start()
                return c
            lax.fori_loop(0, NT_, last, 0)
        return carry
    lax.fori_loop(0, 2, rep, 0)
    for t in range(NT_):
        for i in range(2):
            o_copy(t, i).wait()


@jax.jit
def pallas_interleave_layers__linear_attn_block__mha_block__prompt_kernel(
    A_x: jax.Array,
    A_wqkv: jax.Array,
    A_wo: jax.Array,
    B_x: jax.Array,
    B_wqkv: jax.Array,
    B_wo: jax.Array,
):
    del B_x
    x = A_x.reshape(S, D)
    out = pl.pallas_call(
        _kernel,
        out_shape=jax.ShapeDtypeStruct((S, D), A_x.dtype),
        in_specs=[pl.BlockSpec(memory_space=pl.ANY)] * 5,
        out_specs=pl.BlockSpec(memory_space=pl.ANY),
        scratch_shapes=[
            pltpu.VMEM((S, D), BF16),
            pltpu.VMEM((D, 3 * D), BF16),
            pltpu.VMEM((D, D), BF16),
            pltpu.VMEM((D, 3 * D), BF16),
            pltpu.VMEM((D, D), BF16),
            pltpu.VMEM((S, D), F32),
            pltpu.VMEM((D, D), I32),
            pltpu.VMEM((3 * D // 2, D), I32),
            pltpu.VMEM((H, S // 4, LANE), I32),
            pltpu.VMEM((32 * H, S), I32),
            pltpu.VMEM((NG, TM + 32, LANE), F32),
            pltpu.VMEM((S // 2, D), I32),
            pltpu.VMEM((D, S), F32),
            pltpu.VMEM((2, D, LANE), F32),
            pltpu.VMEM((5, D, LANE), F32),
            pltpu.VMEM((H, S), I32),
            pltpu.VMEM((D, S), F32),
            pltpu.VMEM((D, S), F32),
            pltpu.VMEM((2 * UNROLL, S, TQ), F32),
            pltpu.VMEM((D, D), F32),
            pltpu.VMEM((D, LANE), F32),
            pltpu.VMEM((H, S), F32),
            pltpu.VMEM((D // 2, D), I32),
            pltpu.VMEM((24, TQ), F32),
            pltpu.SemaphoreType.DMA((NT_,)),
            pltpu.SemaphoreType.DMA((6,)),
            pltpu.SemaphoreType.DMA((2 * NT_,)),
        ],
        compiler_params=pltpu.CompilerParams(vmem_limit_bytes=110 * 1024 * 1024),
    )(x, A_wqkv, A_wo, B_wqkv, B_wo)
    return out.reshape(A_x.shape)
```
